```python
import jax
import jax.numpy as jnp

def _softmax(x, axis=-1):
    return jax.nn.softmax(x, axis=axis)
def _gelu(x):
    return jax.nn.gelu(x, approximate=True)
def _silu(x):
    return jax.nn.silu(x)
def _sigmoid(x):
    return jax.nn.sigmoid(x)
def _layernorm(x, axis=-1, eps=1e-5):
    m = jnp.mean(x, axis=axis, keepdims=True)
    v = jnp.var(x, axis=axis, keepdims=True)
    return (x - m) / jnp.sqrt(v + eps)
def _scatter_add(tgt, idx, src, axis=0):
    return tgt.at[idx].add(src)
def _segment_sum(src, seg, n):
    return jax.ops.segment_sum(src, seg, n)
class _Rng:
    def __init__(self, key):
        self._k = key
    def _next(self):
        self._k, sub = jax.random.split(self._k)
        return sub
    def normal(self, shape):
        return jax.random.normal(self._next(), shape, dtype=jnp.bfloat16)
    def randint(self, lo, hi, shape):
        return jax.random.randint(self._next(), shape, lo, hi, dtype=jnp.int32)
    def uniform(self, shape, lo=0.0, hi=1.0):
        return jax.random.uniform(self._next(), shape, jnp.bfloat16, lo, hi)
    def permutation(self, n):
        return jax.random.permutation(self._next(), n)


kernel_name = 'interleave_layers__sliding_block__sliding_local_dilated__prompt'

def setup_inputs():
    _rng = _Rng(jax.random.key(int.from_bytes(__import__("os").urandom(4), "little")))
    _w = (lambda a: (lambda t: t.astype(jnp.bfloat16) if jnp.issubdtype(t.dtype, jnp.floating) else t)(jnp.asarray(a)))
    def _A_setup():
        B, S, D = 1, 2048, 1024
        return {
            "x": _w((lambda *s: _rng.normal(s) * 0.05)(B, S, D)),
            "wqkv": _w((lambda *s: _rng.normal(s) * 0.05)(D, 3 * D)),
            "wo": _w((lambda *s: _rng.normal(s) * 0.05)(D, D)),
        }
    _A_in = _A_setup()

    def _B_setup():
        B, S, D = 1, 2048, 1024
        return {
            "x": _w((lambda *s: _rng.normal(s) * 0.05)(B, S, D)),
            "wqkv": _w((lambda *s: _rng.normal(s) * 0.05)(D, 3 * D)),
            "wo": _w((lambda *s: _rng.normal(s) * 0.05)(D, D)),
        }
    _B_in = _B_setup()

    return {
        "A_x": _A_in["x"],
        "A_wqkv": _A_in["wqkv"],
        "A_wo": _A_in["wo"],
        "B_x": _B_in["x"],
        "B_wqkv": _B_in["wqkv"],
        "B_wo": _B_in["wo"],
    }

def reference(A_x, A_wqkv, A_wo, B_x, B_wqkv, B_wo):
    def _A_ref(x, wqkv, wo):
        B, S, D = x.shape
        H = 32; Dh = D // H; W = 256
        qkv = (lambda x, *d: x.transpose(*d))((x @ wqkv).reshape(B, S, 3, H, Dh), 2, 0, 3, 1, 4)
        q, k, v = qkv[0], qkv[1], qkv[2]
        scores = jnp.einsum("bhqd,bhkd->bhqk", q, k) * (Dh ** -0.5)
        idx = jnp.arange(S)
        mask = (idx[:, None] - idx[None, :] >= 0) & (idx[:, None] - idx[None, :] < W)
        scores = jnp.where(mask[None, None], scores, -1e9)
        p = _softmax(scores, axis=-1)
        o = jnp.einsum("bhqk,bhkd->bhqd", p, v)
        return (lambda x, *d: x.transpose(*d))(o, 0, 2, 1, 3).reshape(B, S, D) @ wo

    def _B_ref(x, wqkv, wo):
        B, S, D = x.shape
        H = 32; Dh = D // H
        W, dil = 8, 2
        qkv = (lambda x, *d: x.transpose(*d))((x @ wqkv).reshape(B, S, 3, H, Dh), 2, 0, 3, 1, 4)
        q, k, v = qkv[0], qkv[1], qkv[2]
        scale = Dh ** -0.5
        pos = jnp.arange(S)
        off = jnp.arange(W) * dil
        idx = pos[:, None] - off[None, :]
        mask = idx >= 0
        idx_c = jnp.where(mask, idx, 0).reshape(-1)
        kg = k[:, :, idx_c, :].reshape(B, H, S, W, Dh)
        vg = v[:, :, idx_c, :].reshape(B, H, S, W, Dh)
        logits = jnp.einsum("bhsd,bhswd->bhsw", q, kg) * scale
        logits = jnp.where(mask[None, None, :, :], logits, -1e9)
        attn = _softmax(logits, axis=-1)
        o = jnp.einsum("bhsw,bhswd->bhsd", attn, vg)
        return (lambda x, *d: x.transpose(*d))(o, 0, 2, 1, 3).reshape(B, S, D) @ wo

    x = A_x
    x = x + _A_ref(_layernorm(x, axis=-1), A_wqkv, A_wo)
    x = x + _B_ref(_layernorm(x, axis=-1), B_wqkv, B_wo)
    x = x + _A_ref(_layernorm(x, axis=-1), A_wqkv, A_wo)
    x = x + _B_ref(_layernorm(x, axis=-1), B_wqkv, B_wo)
    return x
```

```python
import functools, math
import numpy as np
import jax
import jax.numpy as jnp
from jax import lax
from jax.experimental import pallas as pl
from jax.experimental.pallas import tpu as pltpu

S, D, H, DH = 2048, 1024, 32, 32
T = 128
NT = (((1,), (1,)), ((), ()))
NN = (((1,), (0,)), ((), ()))
TN = (((0,), (0,)), ((), ()))
NEG = -1e30
F32 = jnp.float32
BF16 = jnp.bfloat16
QSCALE = float(DH ** -0.5 * math.log2(math.e))


def _make(BM=512, SKEW=1, NL=4):
    NSUB = BM // T
    NB = S // T

    def layernorm(x):
        m = jnp.mean(x, axis=-1, keepdims=True)
        xc = x - m
        v = jnp.mean(xc * xc, axis=-1, keepdims=True)
        return xc * lax.rsqrt(v + 1e-5)

    def kernel(x_ref, wqkvA, woA, wqkvB, woB, out_ref,
               x_s, q_s, o_s, k_all, vt_all, wvt):
        t = pl.program_id(0)

        @pl.when(t == 0)
        def _():
            for li, w in enumerate((wqkvA, wqkvB)):
                for c in range(D // 256):
                    wv = w[:, 2 * D + c * 256: 2 * D + (c + 1) * 256].astype(F32)
                    wvt[li, c * 256:(c + 1) * 256, :] = wv.T.astype(BF16)
            for l in range(4):
                k_all[l, 0:2 * T, :] = jnp.zeros((2 * T, D), BF16)
                vt_all[l, 0] = jnp.zeros((D, T), BF16)
                vt_all[l, 1] = jnp.zeros((D, T), BF16)

        x_s[...] = x_ref[...].astype(F32)

        row = lax.broadcasted_iota(jnp.int32, (T, T), 0)
        col = lax.broadcasted_iota(jnp.int32, (T, T), 1)
        tri = row <= col
        lane_head = lax.broadcasted_iota(jnp.int32, (T // 2, T), 1) // DH
        hmask = [jnp.where(lane_head == h, jnp.uint32(0xFFFFFFFF), jnp.uint32(0)) for h in range(4)]
        row4 = lax.broadcasted_iota(jnp.int32, (T, 4 * T), 0)
        col4 = lax.broadcasted_iota(jnp.int32, (T, 4 * T), 1) & (T - 1)
        tri4 = row4 <= col4
        rowp = lax.broadcasted_iota(jnp.int32, (T // 2, 4 * T), 0) * 2
        colp = lax.broadcasted_iota(jnp.int32, (T // 2, 4 * T), 1) & (T - 1)
        trimask = (jnp.where(rowp <= colp, jnp.uint32(0xFFFF), jnp.uint32(0)) |
                   jnp.where(rowp + 1 <= colp, jnp.uint32(0xFFFF0000), jnp.uint32(0)))

        for l in range(NL):
            isA = (l % 2 == 0)
            wqkv = wqkvA if isA else wqkvB
            wo = woA if isA else woB
            li = 0 if isA else 1
            ln = layernorm(x_s[...]).astype(BF16)
            q = jnp.dot(ln, wqkv[:, 0:D], preferred_element_type=F32)
            q_s[...] = (q * QSCALE).astype(BF16)
            k = jnp.dot(ln, wqkv[:, D:2 * D], preferred_element_type=F32)
            k_all[l, pl.ds(pl.multiple_of((t * NSUB + 2) * T, T), BM), :] = k.astype(BF16)
            vt = lax.dot_general(wvt[li], ln, NT, preferred_element_type=F32).astype(BF16)
            for a in range(NSUB):
                vt_all[l, t * NSUB + 2 + a] = vt[:, a * T:(a + 1) * T]

            units = [(a, g) for a in range(NSUB) for g in range(D // T)]

            def s1(u):
                a, g = u
                ag = t * NSUB + a
                q4 = pltpu.bitcast(q_s[a * T:(a + 1) * T, g * T:(g + 1) * T], jnp.uint32)
                qm = jnp.concatenate([q4 & hmask[h] for h in range(4)], axis=0)
                qm = pltpu.bitcast(qm, BF16)
                if isA:
                    k4 = k_all[l, pl.ds(pl.multiple_of(ag * T, T), 3 * T), g * T:(g + 1) * T]
                else:
                    k4 = k_all[l, pl.ds(pl.multiple_of((ag + 2) * T - 16, 16), T + 16), g * T:(g + 1) * T]
                return lax.dot_general(k4, qm, NT, preferred_element_type=F32)

            def s2(u, st):
                a, g = u
                ag = t * NSUB + a
                if isA:
                    bias_far = jnp.where(ag >= 2, 0.0, NEG).astype(F32)
                    bias_mid = jnp.where(ag >= 1, 0.0, NEG).astype(F32)
                    sm = jnp.where(tri4, st[2 * T:], st[:T] + bias_far)
                    smid = st[T:2 * T] + bias_mid
                    m = jnp.max(jnp.maximum(sm, smid), axis=0, keepdims=True)
                    pm = jnp.exp2(sm - m)
                    pmid = jnp.exp2(smid - m)
                    lsum = jnp.sum(pm + pmid, axis=0, keepdims=True)
                    pmu = pltpu.bitcast(pm.astype(BF16), jnp.uint32)
                    pcur = pmu & trimask
                    pfar = pmu ^ pcur
                    pp = jnp.concatenate([pltpu.bitcast(pfar, BF16), pmid.astype(BF16), pltpu.bitcast(pcur, BF16)], axis=0)
                else:
                    sm = st + biasB[a]
                    m = jnp.max(sm, axis=0, keepdims=True)
                    pm = jnp.exp2(sm - m)
                    lsum = jnp.sum(pm, axis=0, keepdims=True)
                    pp = jnp.concatenate([jnp.zeros((T - 16, 4 * T), BF16), pm.astype(BF16)], axis=0)
                return pp, lsum

            def s3(u, pp, lsum):
                a, g = u
                ag = t * NSUB + a
                outs = []
                for h in range(4):
                    r0 = g * T + h * DH
                    if isA:
                        vv = jnp.concatenate([vt_all[l, ag + i, r0:r0 + DH, :] for i in range(3)], axis=1)
                    else:
                        vv = jnp.concatenate([vt_all[l, ag + 1 + i, r0:r0 + DH, :] for i in range(2)], axis=1)
                    ot = jnp.dot(vv, pp[:, h * T:(h + 1) * T], preferred_element_type=F32)
                    outs.append(ot * (1.0 / lsum[:, h * T:(h + 1) * T]))
                ot4 = jnp.concatenate(outs, axis=0)
                o_s[a * T:(a + 1) * T, g * T:(g + 1) * T] = ot4.T.astype(BF16)

            if not isA:
                biasB = []
                for a in range(NSUB):
                    ag = t * NSUB + a
                    jj = lax.broadcasted_iota(jnp.int32, (T + 16, 4 * T), 0)
                    ii = lax.broadcasted_iota(jnp.int32, (T + 16, 4 * T), 1) & (T - 1)
                    diff = ii - jj + 16
                    validB = (diff >= 0) & (diff <= 14) & ((diff & 1) == 0) & ((jj >= 16) | (ag >= 1))
                    biasB.append(jnp.where(validB, 0.0, NEG).astype(F32))
            if SKEW == 0:
                for u in units:
                    s3(u, *s2(u, s1(u)))
            else:
                nxt = s1(units[0])
                for i, u in enumerate(units):
                    st = nxt
                    if SKEW == 1 and i + 1 < len(units):
                        nxt = s1(units[i + 1])
                    pl_ = s2(u, st)
                    if SKEW == 2 and i + 1 < len(units):
                        nxt = s1(units[i + 1])
                    s3(u, *pl_)

            x_s[...] = x_s[...] + jnp.dot(o_s[...], wo[...], preferred_element_type=F32)

        out_ref[...] = x_s[...].astype(out_ref.dtype)

    def run(A_x, A_wqkv, A_wo, B_x, B_wqkv, B_wo):
        x = A_x.reshape(S, D)
        full = lambda shape: pl.BlockSpec(shape, lambda i: (0, 0), pipeline_mode=pl.Buffered(1))
        out = pl.pallas_call(
            kernel,
            grid=(S // BM,),
            in_specs=[pl.BlockSpec((BM, D), lambda i: (i, 0)),
                      full((D, 3 * D)), full((D, D)), full((D, 3 * D)), full((D, D))],
            out_specs=pl.BlockSpec((BM, D), lambda i: (i, 0)),
            out_shape=jax.ShapeDtypeStruct((S, D), A_x.dtype),
            scratch_shapes=[
                pltpu.VMEM((BM, D), F32), pltpu.VMEM((BM, D), BF16), pltpu.VMEM((BM, D), BF16),
                pltpu.VMEM((4, (NB + 2) * T, D), BF16), pltpu.VMEM((4, NB + 2, D, T), BF16),
                pltpu.VMEM((2, D, D), BF16)],
            compiler_params=pltpu.CompilerParams(
                dimension_semantics=("arbitrary",), vmem_limit_bytes=110 * 1024 * 1024),
        )(x, A_wqkv, A_wo, B_wqkv, B_wo)
        return out.reshape(1, S, D)
    return run


@jax.jit
def pallas_interleave_layers__sliding_block__sliding_local_dilated__prompt_kernel(
    A_x, A_wqkv, A_wo, B_x, B_wqkv, B_wo):
    return _make()(A_x, A_wqkv, A_wo, B_x, B_wqkv, B_wo)
```

```python
import functools, math
import numpy as np
import jax
import jax.numpy as jnp
from jax import lax
from jax.experimental import pallas as pl
from jax.experimental.pallas import tpu as pltpu

S, D, H, DH = 2048, 1024, 32, 32
T = 128
NT = (((1,), (1,)), ((), ()))
NEG = -1e30
F32 = jnp.float32
BF16 = jnp.bfloat16
U32 = jnp.uint32
QSCALE = float(DH ** -0.5 * math.log2(math.e))


def merge(*lists):
    lists = [l for l in lists if l]
    tot = [sum(c for c, _ in l) for l in lists]
    pos = [0] * len(lists)
    acc = [0.0] * len(lists)
    out = []
    while any(p < len(l) for p, l in zip(pos, lists)):
        best = min((acc[i] / tot[i], i) for i in range(len(lists)) if pos[i] < len(lists[i]))[1]
        c, f = lists[best][pos[best]]
        acc[best] += c
        pos[best] += 1
        out.append((c, f))
    return out


def _make(BM=256, NC=512, MODE=1, FLAGS=None, RB=16):
    NSUB = BM // T
    NB = S // T
    NG = D // T

    def layernorm(x):
        m = jnp.mean(x, axis=-1, keepdims=True)
        xc = x - m
        v = jnp.mean(xc * xc, axis=-1, keepdims=True)
        return xc * lax.rsqrt(v + 1e-5)

    def kernel(x_ref, wqkvA_h, woA_h, wqkvB_h, woB_h, out_ref,
               wqkv_s, wo_s, x_s, ln_s, q_s, o_s, k_all, vt_all, qB, kB, vB, tmp, sems):
        t = pl.program_id(0)

        def copy(i):
            src = (wqkvA_h, woA_h, wqkvB_h, woB_h)[i]
            dst = (wqkv_s, wo_s)[i % 2].at[i // 2]
            return pltpu.make_async_copy(src, dst, sems.at[i])

        @pl.when(t == 0)
        def _():
            for i in range(4):
                copy(i).start()
            for l in range(2):
                k_all[l, 0:2 * T, :] = jnp.zeros((2 * T, D), BF16)
                vt_all[l, 0] = jnp.zeros((D, T), BF16)
                vt_all[l, 1] = jnp.zeros((D, T), BF16)
                for e in range(NG):
                    kB[l, e, 0:16, :] = jnp.zeros((16, T), F32)
                    vB[l, e, 0:16, :] = jnp.zeros((16, T), F32)

        x_s[...] = x_ref[...].astype(F32)

        lane_head = lax.broadcasted_iota(jnp.int32, (T // 2, T), 1) // DH
        hmask = [jnp.where(lane_head == h, U32(0xFFFFFFFF), U32(0)) for h in range(4)]
        row4 = lax.broadcasted_iota(jnp.int32, (T, 4 * T), 0)
        col4 = lax.broadcasted_iota(jnp.int32, (T, 4 * T), 1) & (T - 1)
        tri4 = row4 <= col4

        def rows(a, n=1):
            return slice(a * T, (a + n) * T)

        def t_ln(a):
            def f():
                ln_s[rows(a), :] = layernorm(x_s[rows(a), :]).astype(BF16)
            return [(200, f)]

        def t_proj(r, li, a, n=1):
            l = r
            tasks = []
            for c in range(3 * D // NC):
                def f(c=c):
                    y = jnp.dot(ln_s[rows(a, n), :], wqkv_s[li, :, c * NC:(c + 1) * NC], preferred_element_type=F32)
                    ag = t * NSUB + a
                    if li == 1:
                        which = c * NC // D
                        for i in range(NC // T):
                            e = (c * NC % D) // T + i
                            yy = y[:, i * T:(i + 1) * T]
                            if which == 0:
                                qB[e, rows(a, n), :] = yy * QSCALE
                            elif which == 1:
                                kB[r, e, 16 + a * T:16 + (a + n) * T, :] = yy
                            else:
                                vB[r, e, 16 + a * T:16 + (a + n) * T, :] = yy
                    elif c * NC < D:
                        q_s[rows(a, n), c * NC:(c + 1) * NC] = (y * QSCALE).astype(BF16)
                    elif c * NC < 2 * D:
                        k_all[l, pl.ds(pl.multiple_of((ag + 2) * T, T), n * T), c * NC - D:(c + 1) * NC - D] = y.astype(BF16)
                    else:
                        for i in range(n):
                            vt_all[l, ag + 2 + i, c * NC - 2 * D:(c + 1) * NC - 2 * D, :] = y[i * T:(i + 1) * T].T.astype(BF16)
                tasks.append((2 * NC, f))
            return tasks

        def t_out(li, a, n=1):
            tasks = []
            for c in range(D // NC):
                def f(c=c):
                    cs = slice(c * NC, (c + 1) * NC)
                    x_s[rows(a, n), cs] = x_s[rows(a, n), cs] + jnp.dot(o_s[rows(a, n), :], wo_s[li, :, cs], preferred_element_type=F32)
                tasks.append((2 * NC, f))
            return tasks

        def t_attB(r, a):
            tasks = []
            for rg in range(T // RB):
                def f(rg=rg):
                    r0 = a * T + rg * RB
                    qs = [qB[e, r0:r0 + RB, :] for e in range(NG)]
                    Ls = []
                    for w in range(8):
                        R = None
                        for e in range(NG):
                            pr = qs[e] * kB[r, e, pl.ds(r0 + 16 - 2 * w, RB), :]
                            R = pr if R is None else R + pr
                        R = R + pltpu.roll(R, 64, axis=1)
                        R = R + pltpu.roll(R, 32, axis=1)
                        if r0 < 2 * w:
                            pos = lax.broadcasted_iota(jnp.int32, (RB, T), 0) + (t * BM + (r0 - 2 * w))
                            R = jnp.where(pos >= 0, R, NEG)
                        Ls.append(R)
                    m = functools.reduce(jnp.maximum, Ls)
                    ps = [jnp.exp2(L - m) for L in Ls]
                    rl = 1.0 / functools.reduce(jnp.add, ps)
                    ps = [p * rl for p in ps]
                    for e in range(NG):
                        o = None
                        for w in range(8):
                            pr = ps[w] * vB[r, e, pl.ds(r0 + 16 - 2 * w, RB), :]
                            o = pr if o is None else o + pr
                        o_s[r0:r0 + RB, e * T:(e + 1) * T] = o.astype(BF16)
                tasks.append((100, f))
            if a == NSUB - 1:
                def g():
                    for e in range(NG):
                        kB[r, e, 0:16, :] = kB[r, e, BM:BM + 16, :]
                        vB[r, e, 0:16, :] = vB[r, e, BM:BM + 16, :]
                tasks.append((1, g))
            return tasks

        def permute_B():
            def mat(m, _):
                c0 = pl.multiple_of(m * D, D)
                for i in range(NG):
                    wt = wqkv_s[1, i * T:(i + 1) * T, pl.ds(c0, D)].astype(F32).T
                    for h in range(H):
                        tmp[pl.ds(h * 33, DH), :] = wt[h * DH:(h + 1) * DH]
                    pm = jnp.concatenate([tmp[pl.ds(d, H, stride=33), :] for d in range(DH)], axis=0)
                    wqkv_s[1, i * T:(i + 1) * T, pl.ds(c0, D)] = pm.T.astype(BF16)
                return 0
            lax.fori_loop(0, 3, mat, 0)
            def wo(i, _):
                c0 = pl.multiple_of(i * T, T)
                wt = wo_s[1, :, pl.ds(c0, T)].astype(F32)
                for h in range(H):
                    tmp[pl.ds(h * 33, DH), :] = wt[h * DH:(h + 1) * DH]
                pm = jnp.concatenate([tmp[pl.ds(d, H, stride=33), :] for d in range(DH)], axis=0)
                wo_s[1, :, pl.ds(c0, T)] = pm.astype(BF16)
                return 0
            lax.fori_loop(0, NG, wo, 0)

        def t_att(r, li, a):
            if li == 1:
                return t_attB(r, a)
            isA = li == 0
            l = r
            st_ = {}
            pp_ = {}
            cst = {}

            def s1(g):
                ag = t * NSUB + a
                q4 = pltpu.bitcast(q_s[rows(a), g * T:(g + 1) * T], U32)
                qm = jnp.concatenate([q4 & hmask[h] for h in range(4)], axis=0)
                qm = pltpu.bitcast(qm, BF16)
                if isA:
                    k4 = k_all[l, pl.ds(pl.multiple_of(ag * T, T), 3 * T), g * T:(g + 1) * T]
                else:
                    k4 = k_all[l, pl.ds(pl.multiple_of((ag + 2) * T - 16, 16), T + 16), g * T:(g + 1) * T]
                st_[g] = lax.dot_general(k4, qm, NT, preferred_element_type=F32)

            def s2(g):
                ag = t * NSUB + a
                st = st_.pop(g)
                if isA:
                    bias_far = jnp.where(ag >= 2, 0.0, NEG).astype(F32)
                    bias_mid = jnp.where(ag >= 1, 0.0, NEG).astype(F32)
                    sm = jnp.where(tri4, st[2 * T:], st[:T] + bias_far)
                    smid = st[T:2 * T] + bias_mid
                    m = jnp.max(jnp.maximum(sm, smid), axis=0, keepdims=True)
                    pm = jnp.exp2(sm - m)
                    pmid = jnp.exp2(smid - m)
                    lsum = jnp.sum(pm + pmid, axis=0, keepdims=True)
                    pcur = jnp.where(tri4, pm, 0.0)
                    pfar = jnp.where(tri4, 0.0, pm)
                    pp = [jnp.concatenate([pfar[:, h * T:(h + 1) * T], pmid[:, h * T:(h + 1) * T], pcur[:, h * T:(h + 1) * T]], axis=0).astype(BF16) for h in range(4)]
                else:
                    if "b" not in cst:
                        jj = lax.broadcasted_iota(jnp.int32, (T + 16, 4 * T), 0)
                        ii = lax.broadcasted_iota(jnp.int32, (T + 16, 4 * T), 1) & (T - 1)
                        diff = ii - jj + 16
                        validB = (diff >= 0) & (diff <= 14) & ((diff & 1) == 0) & ((jj >= 16) | (ag >= 1))
                        cst["b"] = jnp.where(validB, 0.0, NEG).astype(F32)
                    sm = st + cst["b"]
                    m = jnp.max(sm, axis=0, keepdims=True)
                    pm = jnp.exp2(sm - m)
                    lsum = jnp.sum(pm, axis=0, keepdims=True)
                    pp = [jnp.concatenate([jnp.zeros((T - 16, T), F32), pm[:, h * T:(h + 1) * T]], axis=0).astype(BF16) for h in range(4)]
                pp_[g] = (pp, lsum)

            def s3(g):
                ag = t * NSUB + a
                pp, lsum = pp_.pop(g)
                outs = []
                rl = 1.0 / lsum
                for h in range(4):
                    r0 = g * T + h * DH
                    if isA:
                        vv = jnp.concatenate([vt_all[l, ag + i, r0:r0 + DH, :] for i in range(3)], axis=1)
                    else:
                        vv = jnp.concatenate([vt_all[l, ag + 1 + i, r0:r0 + DH, :] for i in range(2)], axis=1)
                    ot = jnp.dot(vv, pp[h], preferred_element_type=F32)
                    outs.append(ot * rl[:, h * T:(h + 1) * T])
                ot4 = jnp.concatenate(outs, axis=0)
                o_s[rows(a), g * T:(g + 1) * T] = ot4.T.astype(BF16)

            tasks = []
            c1, c2, c3 = (384, 1, 192) if isA else (144, 1, 100)
            for i in range(NG + 2):
                if i < NG:
                    tasks.append((c1, functools.partial(s1, i)))
                if 0 <= i - 1 < NG:
                    tasks.append((c2, functools.partial(s2, i - 1)))
                if 0 <= i - 2 < NG:
                    tasks.append((c3, functools.partial(s3, i - 2)))
            return tasks

        def wait(r, li):
            def f():
                @pl.when(jnp.logical_and(t == 0, r == 0))
                def _():
                    copy(2 * li).wait()
                    copy(2 * li + 1).wait()
                    if li == 1:
                        permute_B()
            return [(1, f)]

        def body(r, _):
            if MODE == 0:
                seq = []
                for li in range(2):
                    seq += wait(r, li)
                    for a in range(NSUB):
                        seq += t_ln(a) + t_proj(r, li, a)
                    for a in range(NSUB):
                        seq += t_att(r, li, a)
                    for a in range(NSUB):
                        seq += t_out(li, a)
            elif MODE == 2:
                seq = []
                for li in range(2):
                    seq += wait(r, li)
                    for a in range(NSUB):
                        seq += t_ln(a)
                    seq += t_proj(r, li, 0, NSUB)
                    for a in range(NSUB):
                        seq += t_att(r, li, a)
                    seq += t_out(li, 0, NSUB)
            elif MODE == 3:
                seq = []
                for li in range(2):
                    seq += wait(r, li)
                    for a in range(NSUB):
                        seq += t_ln(a)
                    seq += t_proj(r, li, 0, NSUB)
                    seq += t_att(r, li, 0) + merge(t_att(r, li, 1), t_out(li, 0)) + t_out(li, 1)
            elif MODE == 4:
                seq = []
                for li in range(2):
                    seq += wait(r, li)
                    for a in range(NSUB):
                        seq += t_ln(a) + t_proj(r, li, a)
                    seq += t_att(r, li, 0) + merge(t_att(r, li, 1), t_out(li, 0)) + t_out(li, 1)
            else:
                seq = wait(r, 0) + t_ln(0) + merge(t_proj(r, 0, 0), t_ln(1))
                seq += merge(t_proj(r, 0, 1), t_att(r, 0, 0))
                seq += wait(r, 1)
                seq += merge(t_out(0, 0) + t_ln(0) + t_proj(r, 1, 0), t_att(r, 0, 1))
                seq += merge(t_out(0, 1) + t_ln(1) + t_proj(r, 1, 1), t_att(r, 1, 0))
                seq += merge(t_out(1, 0), t_att(r, 1, 1))
                seq += t_out(1, 1)
            for _, f in seq:
                f()
            return 0
        lax.fori_loop(0, 2, body, 0)
        out_ref[...] = x_s[...].astype(out_ref.dtype)

    def run(A_x, A_wqkv, A_wo, B_x, B_wqkv, B_wo):
        x = A_x.reshape(S, D)
        anyspec = pl.BlockSpec(memory_space=pl.ANY)
        kw = {}
        if FLAGS:
            kw["flags"] = FLAGS
        out = pl.pallas_call(
            kernel,
            grid=(S // BM,),
            in_specs=[pl.BlockSpec((BM, D), lambda i: (i, 0)), anyspec, anyspec, anyspec, anyspec],
            out_specs=pl.BlockSpec((BM, D), lambda i: (i, 0)),
            out_shape=jax.ShapeDtypeStruct((S, D), A_x.dtype),
            scratch_shapes=[
                pltpu.VMEM((2, D, 3 * D), BF16), pltpu.VMEM((2, D, D), BF16),
                pltpu.VMEM((BM, D), F32), pltpu.VMEM((BM, D), BF16), pltpu.VMEM((BM, D), BF16), pltpu.VMEM((BM, D), BF16),
                pltpu.VMEM((2, (NB + 2) * T, D), BF16), pltpu.VMEM((2, NB + 2, D, T), BF16),
                pltpu.VMEM((NG, BM, T), F32), pltpu.VMEM((2, NG, BM + 16, T), F32), pltpu.VMEM((2, NG, BM + 16, T), F32),
                pltpu.VMEM((33 * H, T), F32),
                pltpu.SemaphoreType.DMA((4,))],
            compiler_params=pltpu.CompilerParams(
                dimension_semantics=("arbitrary",), vmem_limit_bytes=110 * 1024 * 1024, **kw),
        )(x, A_wqkv, A_wo, B_wqkv, B_wo)
        return out.reshape(1, S, D)
    return run


@jax.jit
def pallas_interleave_layers__sliding_block__sliding_local_dilated__prompt_kernel(
    A_x, A_wqkv, A_wo, B_x, B_wqkv, B_wo):
    return _make(MODE=0)(A_x, A_wqkv, A_wo, B_x, B_wqkv, B_wo)
```

```python
import functools, math
import numpy as np
import jax
import jax.numpy as jnp
from jax import lax
from jax.experimental import pallas as pl
from jax.experimental.pallas import tpu as pltpu

S, D, H, DH = 2048, 1024, 32, 32
T = 128
NT = (((1,), (1,)), ((), ()))
NEG = -1e30
F32 = jnp.float32
BF16 = jnp.bfloat16
U32 = jnp.uint32
QSCALE = float(DH ** -0.5 * math.log2(math.e))


def merge(*lists):
    lists = [l for l in lists if l]
    tot = [sum(c for c, _ in l) for l in lists]
    pos = [0] * len(lists)
    acc = [0.0] * len(lists)
    out = []
    while any(p < len(l) for p, l in zip(pos, lists)):
        best = min((acc[i] / tot[i], i) for i in range(len(lists)) if pos[i] < len(lists[i]))[1]
        c, f = lists[best][pos[best]]
        acc[best] += c
        pos[best] += 1
        out.append((c, f))
    return out


def _make(BM=256, NC=512, MODE=1, FLAGS=None, RB=16, SEG=0, LAG=2, NS=8, UNI=1, MB=1, PP=0):
    NSUB = BM // T
    NB = S // T
    NG = D // T

    def layernorm(x):
        m = jnp.mean(x, axis=-1, keepdims=True)
        xc = x - m
        v = jnp.mean(xc * xc, axis=-1, keepdims=True)
        return xc * lax.rsqrt(v + 1e-5)

    def kernel(x_ref, wqkvA_h, woA_h, wqkvB_h, woB_h, out_ref,
               wqkv_s, wo_s, x_s, ln_s, q_s, o_s, k_all, vt_all, qB, kB, vB, tmp, wBT, sems):
        t = pl.program_id(0)

        def copy(i):
            if i < 6:
                li, m = 1 - i // 3, i % 3
                return pltpu.make_async_copy((wqkvA_h, wqkvB_h)[li].at[:, m * D:(m + 1) * D],
                                             wqkv_s.at[li, :, m * D:(m + 1) * D], sems.at[i])
            li = i - 6
            return pltpu.make_async_copy((woA_h, woB_h)[li], wo_s.at[li], sems.at[i])

        @pl.when(t == 0)
        def _():
            for i in (3, 4, 5, 6, 0, 1, 2, 7):
                copy(i).start()
            for l in range(2):
                k_all[l, 0:2 * T, :] = jnp.zeros((2 * T, D), BF16)
                vt_all[l, 0] = jnp.zeros((D, T), BF16)
                vt_all[l, 1] = jnp.zeros((D, T), BF16)
                for e in range(NG):
                    kB[l, e, 0:16, :] = jnp.zeros((16, T), F32)
                    vB[l, e, 0:16, :] = jnp.zeros((16, T), F32)

        x_s[...] = x_ref[...].astype(F32)

        lane_head = lax.broadcasted_iota(jnp.int32, (T // 2, T), 1) // DH
        hmask = [jnp.where(lane_head == h, U32(0xFFFFFFFF), U32(0)) for h in range(4)]
        row4 = lax.broadcasted_iota(jnp.int32, (T, 4 * T), 0)
        col4 = lax.broadcasted_iota(jnp.int32, (T, 4 * T), 1) & (T - 1)
        tri4 = row4 <= col4

        def rows(a, n=1):
            return slice(a * T, (a + n) * T)

        def t_ln(a):
            def f():
                ln_s[rows(a), :] = layernorm(x_s[rows(a), :]).astype(BF16)
            return [(200, f)]

        def t_proj(r, li, a, n=1):
            l = r
            tasks = []
            for c in range(3 * D // NC):
                def f(c=c):
                    if li == 0:
                        y = jnp.dot(ln_s[rows(a, n), :], wqkv_s[li, :, c * NC:(c + 1) * NC], preferred_element_type=F32)
                    else:
                        y = lax.dot_general(ln_s[rows(a, n), :], wBT[c * NC:(c + 1) * NC, :], NT, preferred_element_type=F32)
                    ag = t * NSUB + a
                    if li == 1:
                        which = c * NC // D
                        for i in range(NC // T):
                            e = (c * NC % D) // T + i
                            yy = y[:, i * T:(i + 1) * T]
                            if which == 0:
                                qB[e, rows(a, n), :] = yy * QSCALE
                            elif which == 1:
                                kB[r, e, 16 + a * T:16 + (a + n) * T, :] = yy
                            else:
                                vB[r, e, 16 + a * T:16 + (a + n) * T, :] = yy
                    elif c * NC < D:
                        q_s[rows(a, n), c * NC:(c + 1) * NC] = (y * QSCALE).astype(BF16)
                    elif c * NC < 2 * D:
                        k_all[l, pl.ds(pl.multiple_of((ag + 2) * T, T), n * T), c * NC - D:(c + 1) * NC - D] = y.astype(BF16)
                    else:
                        for i in range(n):
                            vt_all[l, ag + 2 + i, c * NC - 2 * D:(c + 1) * NC - 2 * D, :] = y[i * T:(i + 1) * T].T.astype(BF16)
                tasks.append((2 * NC, f))
            return tasks

        def t_out(li, a, n=1):
            tasks = []
            for c in range(D // NC):
                def f(c=c):
                    cs = slice(c * NC, (c + 1) * NC)
                    x_s[rows(a, n), cs] = x_s[rows(a, n), cs] + jnp.dot(o_s[rows(a, n), :], wo_s[li, :, cs], preferred_element_type=F32)
                tasks.append((2 * NC, f))
            return tasks

        def t_attB(r, a):
            tasks = []
            for rg in range(T // RB):
                def f(rg=rg):
                    r0 = a * T + rg * RB
                    qs = [qB[e, r0:r0 + RB, :] for e in range(NG)]
                    Ls = []
                    for w in range(8):
                        R = None
                        for e in range(NG):
                            pr = qs[e] * kB[r, e, pl.ds(r0 + 16 - 2 * w, RB), :]
                            R = pr if R is None else R + pr
                        R = R + pltpu.roll(R, 64, axis=1)
                        R = R + pltpu.roll(R, 32, axis=1)
                        if r0 < 2 * w:
                            pos = lax.broadcasted_iota(jnp.int32, (RB, T), 0) + (t * BM + (r0 - 2 * w))
                            R = jnp.where(pos >= 0, R, NEG)
                        Ls.append(R)
                    m = functools.reduce(jnp.maximum, Ls)
                    ps = [jnp.exp2(L - m) for L in Ls]
                    rl = 1.0 / functools.reduce(jnp.add, ps)
                    ps = [p * rl for p in ps]
                    for e in range(NG):
                        o = None
                        for w in range(8):
                            pr = ps[w] * vB[r, e, pl.ds(r0 + 16 - 2 * w, RB), :]
                            o = pr if o is None else o + pr
                        o_s[r0:r0 + RB, e * T:(e + 1) * T] = o.astype(BF16)
                tasks.append((100, f))
            if a == NSUB - 1:
                def g():
                    for e in range(NG):
                        kB[r, e, 0:16, :] = kB[r, e, BM:BM + 16, :]
                        vB[r, e, 0:16, :] = vB[r, e, BM:BM + 16, :]
                tasks.append((1, g))
            return tasks

        def perm_rows(wt, j):
            for h in range(H):
                tmp[j, pl.ds(h * 33, DH), :] = wt[h * DH:(h + 1) * DH]
            return jnp.concatenate([tmp[j, pl.ds(d, H, stride=33), :] for d in range(DH)], axis=0)

        def permute_qkv(m):
            c0 = m * D
            for i in range(NG):
                wt = wqkv_s[1, i * T:(i + 1) * T, pl.ds(c0, D)].astype(F32).T
                wBT[pl.ds(c0, D), i * T:(i + 1) * T] = perm_rows(wt, i % 4).astype(BF16)

        def permute_o():
            for i in range(NG):
                wo_s[1, :, i * T:(i + 1) * T] = perm_rows(wo_s[1, :, i * T:(i + 1) * T].astype(F32), i % 4).astype(BF16)

        def t_att(r, li, a, parts=False):
            if li == 1:
                return t_attB(r, a)
            isA = li == 0
            l = r
            st_ = {}
            pp_ = {}
            cst = {}

            def s1(g):
                ag = t * NSUB + a
                q4 = pltpu.bitcast(q_s[rows(a), g * T:(g + 1) * T], U32)
                qm = jnp.concatenate([q4 & hmask[h] for h in range(4)], axis=0)
                qm = pltpu.bitcast(qm, BF16)
                if isA:
                    k4 = k_all[l, pl.ds(pl.multiple_of(ag * T, T), 3 * T), g * T:(g + 1) * T]
                else:
                    k4 = k_all[l, pl.ds(pl.multiple_of((ag + 2) * T - 16, 16), T + 16), g * T:(g + 1) * T]
                st_[g] = lax.dot_general(k4, qm, NT, preferred_element_type=F32)

            def s2(g):
                ag = t * NSUB + a
                st = st_.pop(g)
                if isA:
                    bias_far = jnp.where(ag >= 2, 0.0, NEG).astype(F32)
                    bias_mid = jnp.where(ag >= 1, 0.0, NEG).astype(F32)
                    sm = jnp.where(tri4, st[2 * T:], st[:T] + bias_far)
                    smid = st[T:2 * T]
                    m = jnp.maximum(jnp.max(sm, axis=0, keepdims=True), jnp.max(smid, axis=0, keepdims=True) + bias_mid)
                    pm = jnp.exp2(sm - m)
                    pmid = jnp.exp2(smid - (m - bias_mid))
                    lsum = jnp.sum(pm + pmid, axis=0, keepdims=True)
                    pcur = jnp.where(tri4, pm, 0.0)
                    pfar = jnp.where(tri4, 0.0, pm)
                    pp = [jnp.concatenate([pfar[:, h * T:(h + 1) * T], pmid[:, h * T:(h + 1) * T], pcur[:, h * T:(h + 1) * T]], axis=0).astype(BF16) for h in range(4)]
                else:
                    if "b" not in cst:
                        jj = lax.broadcasted_iota(jnp.int32, (T + 16, 4 * T), 0)
                        ii = lax.broadcasted_iota(jnp.int32, (T + 16, 4 * T), 1) & (T - 1)
                        diff = ii - jj + 16
                        validB = (diff >= 0) & (diff <= 14) & ((diff & 1) == 0) & ((jj >= 16) | (ag >= 1))
                        cst["b"] = jnp.where(validB, 0.0, NEG).astype(F32)
                    sm = st + cst["b"]
                    m = jnp.max(sm, axis=0, keepdims=True)
                    pm = jnp.exp2(sm - m)
                    lsum = jnp.sum(pm, axis=0, keepdims=True)
                    pp = [jnp.concatenate([jnp.zeros((T - 16, T), F32), pm[:, h * T:(h + 1) * T]], axis=0).astype(BF16) for h in range(4)]
                pp_[g] = (pp, lsum)

            def s3(g):
                ag = t * NSUB + a
                pp, lsum = pp_.pop(g)
                outs = []
                rl = 1.0 / lsum
                for h in range(4):
                    r0 = g * T + h * DH
                    if isA:
                        vv = jnp.concatenate([vt_all[l, ag + i, r0:r0 + DH, :] for i in range(3)], axis=1)
                    else:
                        vv = jnp.concatenate([vt_all[l, ag + 1 + i, r0:r0 + DH, :] for i in range(2)], axis=1)
                    ot = jnp.dot(vv, pp[h], preferred_element_type=F32)
                    outs.append(ot * rl[:, h * T:(h + 1) * T])
                ot4 = jnp.concatenate(outs, axis=0)
                o_s[rows(a), g * T:(g + 1) * T] = ot4.T.astype(BF16)

            def s1p(g, i):
                ag = t * NSUB + a
                if i == 0:
                    q4 = pltpu.bitcast(q_s[rows(a), g * T:(g + 1) * T], U32)
                    qm = jnp.concatenate([q4 & hmask[h] for h in range(4)], axis=0)
                    cst["qm", g] = pltpu.bitcast(qm, BF16)
                k4 = k_all[l, pl.ds(pl.multiple_of((ag + i) * T, T), T), g * T:(g + 1) * T]
                st_[g, i] = lax.dot_general(k4, cst["qm", g], NT, preferred_element_type=F32)

            def s2p(g):
                ag = t * NSUB + a
                bias_far = jnp.where(ag >= 2, 0.0, NEG).astype(F32)
                bias_mid = jnp.where(ag >= 1, 0.0, NEG).astype(F32)
                sm = jnp.where(tri4, st_.pop((g, 2)), st_.pop((g, 0)) + bias_far)
                smid = st_.pop((g, 1)) + bias_mid
                m = jnp.max(jnp.maximum(sm, smid), axis=0, keepdims=True)
                pm = jnp.exp2(sm - m)
                pmid = jnp.exp2(smid - m)
                lsum = jnp.sum(pm + pmid, axis=0, keepdims=True)
                pcur = jnp.where(tri4, pm, 0.0)
                pfar = jnp.where(tri4, 0.0, pm)
                for i, p in enumerate((pfar, pmid, pcur)):
                    pp_[g, i] = [p[:, h * T:(h + 1) * T].astype(BF16) for h in range(4)]
                cst["rl", g] = 1.0 / lsum

            def s3p(g, i):
                ag = t * NSUB + a
                pp = pp_.pop((g, i))
                outs = []
                for h in range(4):
                    r0 = g * T + h * DH
                    ot = jnp.dot(vt_all[l, ag + i, r0:r0 + DH, :], pp[h], preferred_element_type=F32)
                    outs.append(ot if i == 0 else cst["o", g][h] + ot)
                cst["o", g] = outs
                if i == 2:
                    rl = cst["rl", g]
                    ot4 = jnp.concatenate([outs[h] * rl[:, h * T:(h + 1) * T] for h in range(4)], axis=0)
                    o_s[rows(a), g * T:(g + 1) * T] = ot4.T.astype(BF16)

            if parts:
                return s1, s2, s3
            tasks = []
            if SEG:
                for n in range(NG + 2):
                    for i in range(3):
                        if n < NG:
                            tasks.append((128, functools.partial(s1p, n, i)))
                        if i == SEG - 1 and 0 <= n - 1 < NG:
                            tasks.append((1, functools.partial(s2p, n - 1)))
                        if 0 <= n - 2 < NG:
                            tasks.append((64, functools.partial(s3p, n - 2, i)))
                return tasks
            c1, c2, c3 = (384, 1, 192) if isA else (144, 1, 100)
            for i in range(NG + LAG):
                if i < NG:
                    tasks.append((c1, functools.partial(s1, i)))
                if 0 <= i - 1 < NG:
                    tasks.append((c2, functools.partial(s2, i - 1)))
                if 0 <= i - LAG < NG:
                    tasks.append((c3, functools.partial(s3, i - LAG)))
            return tasks

        def wait(r, i):
            def f():
                @pl.when(jnp.logical_and(t == 0, r == 0))
                def _():
                    copy(i).wait()
                    for j in ():
                        copy(j).start()
            return [(1, f)]

        def prepB(r):
            def f():
                @pl.when(jnp.logical_and(t == 0, r == 0))
                def _():
                    for j in (0, 1, 2, 7):
                        copy(j).wait()
                    for m in range(3):
                        permute_qkv(m)
                    permute_o()
            return [(1, f)]

        def body(r, _):
            seq = []
            npm = D // NC
            for li in range(2):
                pr = [t_proj(r, li, a) for a in range(NSUB)]
                if li == 0:
                    seq += t_ln(0)
                    for m in range(3):
                        seq += wait(r, 3 + m)
                        for a in range(NSUB):
                            seq += pr[a][m * npm:(m + 1) * npm]
                            if m == 0 and a + 1 < NSUB:
                                seq += t_ln(a + 1)
                else:
                    if not PP:
                        seq += prepB(r)
                    for a in range(NSUB):
                        seq += t_ln(a) + pr[a]
                if li == 0 and UNI:
                    fs = [t_att(r, li, a, True) for a in range(NSUB)]
                    n = NSUB * NG
                    for i in range(n + LAG):
                        if i < n:
                            seq.append((1, functools.partial(fs[i // NG][0], i % NG)))
                        if 0 <= i - 1 < n:
                            seq.append((1, functools.partial(fs[(i - 1) // NG][1], (i - 1) % NG)))
                        if 0 <= i - LAG < n:
                            seq.append((1, functools.partial(fs[(i - LAG) // NG][2], (i - LAG) % NG)))
                        if PP and i == PP:
                            seq += prepB(r)
                else:
                    for a in range(NSUB):
                        seq += t_att(r, li, a)
                if li == 0:
                    seq += wait(r, 6)
                for a in range(NSUB):
                    seq += t_out(li, a)
            for _, f in seq:
                f()
            return 0
        lax.fori_loop(0, 2, body, 0)
        out_ref[...] = x_s[...].astype(out_ref.dtype)

    def run(A_x, A_wqkv, A_wo, B_x, B_wqkv, B_wo):
        x = A_x.reshape(S, D)
        anyspec = pl.BlockSpec(memory_space=pl.ANY)
        kw = {}
        if FLAGS:
            kw["flags"] = FLAGS
        out = pl.pallas_call(
            kernel,
            grid=(NS,),
            in_specs=[pl.BlockSpec((BM, D), lambda i: (i, 0)), anyspec, anyspec, anyspec, anyspec],
            out_specs=pl.BlockSpec((BM, D), lambda i: (i, 0)),
            out_shape=jax.ShapeDtypeStruct((S, D), A_x.dtype),
            scratch_shapes=[
                pltpu.VMEM((2, D, 3 * D), BF16), pltpu.VMEM((2, D, D), BF16),
                pltpu.VMEM((BM, D), F32), pltpu.VMEM((BM, D), BF16), pltpu.VMEM((BM, D), BF16), pltpu.VMEM((BM, D), BF16),
                pltpu.VMEM((2, (NB + 2) * T, D), BF16), pltpu.VMEM((2, NB + 2, D, T), BF16),
                pltpu.VMEM((NG, BM, T), F32), pltpu.VMEM((2, NG, BM + 16, T), F32), pltpu.VMEM((2, NG, BM + 16, T), F32),
                pltpu.VMEM((4, 33 * H, T), F32), pltpu.VMEM((3 * D, D), BF16),
                pltpu.SemaphoreType.DMA((8,))],
            compiler_params=pltpu.CompilerParams(
                dimension_semantics=("arbitrary",), vmem_limit_bytes=110 * 1024 * 1024, **kw),
        )(x, A_wqkv, A_wo, B_wqkv, B_wo)
        return out.reshape(1, S, D)
    return run


@jax.jit
def pallas_interleave_layers__sliding_block__sliding_local_dilated__prompt_kernel(
    A_x, A_wqkv, A_wo, B_x, B_wqkv, B_wo):
    return _make()(A_x, A_wqkv, A_wo, B_x, B_wqkv, B_wo)
```

```python
import functools, math
import numpy as np
import jax
import jax.numpy as jnp
from jax import lax
from jax.experimental import pallas as pl
from jax.experimental.pallas import tpu as pltpu

S, D, H, DH = 2048, 1024, 32, 32
T = 128
NT = (((1,), (1,)), ((), ()))
NEG = -1e30
F32 = jnp.float32
BF16 = jnp.bfloat16
U32 = jnp.uint32
QSCALE = float(DH ** -0.5 * math.log2(math.e))


def _make(BM=256, NC=512, MODE=1, FLAGS=None, RB=16, SEG=0, LAG=2, NS=8, UNI=1, MB=1, PP=0):
    NSUB = BM // T
    NB = S // T
    NG = D // T

    def layernorm(x):
        m = jnp.mean(x, axis=-1, keepdims=True)
        xc = x - m
        v = jnp.mean(xc * xc, axis=-1, keepdims=True)
        return xc * lax.rsqrt(v + 1e-5)

    def kernel(x_ref, wqkvA_h, woA_h, wqkvB_h, woB_h, out_ref,
               wqkv_s, wo_s, x_s, ln_s, q_s, o_s, k_all, vt_all, qB, kB, vB, tmp, wBT, sems):
        t = pl.program_id(0)

        def copy(i):
            if i >= 8:
                j = (i - 8) % 4
                cs = slice(0, D) if i < 12 else slice(D, 3 * D)
                rs = slice(j * D // 4, (j + 1) * D // 4)
                return pltpu.make_async_copy(wqkvA_h.at[rs, cs], wqkv_s.at[0, rs, cs], sems.at[i])
            if i < 6:
                li, m = 1 - i // 3, i % 3
                return pltpu.make_async_copy((wqkvA_h, wqkvB_h)[li].at[:, m * D:(m + 1) * D],
                                             wqkv_s.at[li, :, m * D:(m + 1) * D], sems.at[i])
            li = i - 6
            return pltpu.make_async_copy((woA_h, woB_h)[li], wo_s.at[li], sems.at[i])

        @pl.when(t == 0)
        def _():
            for i in (8, 9, 10, 11):
                copy(i).start()
            for l in range(2):
                k_all[l, 0:2 * T, :] = jnp.zeros((2 * T, D), BF16)
                vt_all[l, 0] = jnp.zeros((D, T), BF16)
                vt_all[l, 1] = jnp.zeros((D, T), BF16)
                for e in range(NG):
                    kB[l, e, 0:16, :] = jnp.zeros((16, T), F32)
                    vB[l, e, 0:16, :] = jnp.zeros((16, T), F32)

        x_s[...] = x_ref[...].astype(F32)

        lane_head = lax.broadcasted_iota(jnp.int32, (T // 2, T), 1) // DH
        hmask = [jnp.where(lane_head == h, U32(0xFFFFFFFF), U32(0)) for h in range(4)]
        row4 = lax.broadcasted_iota(jnp.int32, (T, 4 * T), 0)
        col4 = lax.broadcasted_iota(jnp.int32, (T, 4 * T), 1) & (T - 1)
        tri4 = row4 <= col4

        def rows(a, n=1):
            return slice(a * T, (a + n) * T)

        def t_ln(a):
            def f():
                ln_s[rows(a), :] = layernorm(x_s[rows(a), :]).astype(BF16)
            return [(200, f)]

        def t_proj(r, li, a, n=1):
            l = r
            tasks = []
            for c in range(3 * D // NC):
                def f(c=c):
                    if li == 0:
                        y = jnp.dot(ln_s[rows(a, n), :], wqkv_s[li, :, c * NC:(c + 1) * NC], preferred_element_type=F32)
                    else:
                        y = lax.dot_general(ln_s[rows(a, n), :], wBT[c * NC:(c + 1) * NC, :], NT, preferred_element_type=F32)
                    ag = t * NSUB + a
                    if li == 1:
                        which = c * NC // D
                        for i in range(NC // T):
                            e = (c * NC % D) // T + i
                            yy = y[:, i * T:(i + 1) * T]
                            if which == 0:
                                qB[e, rows(a, n), :] = yy * QSCALE
                            elif which == 1:
                                kB[r, e, 16 + a * T:16 + (a + n) * T, :] = yy
                            else:
                                vB[r, e, 16 + a * T:16 + (a + n) * T, :] = yy
                    elif c * NC < D:
                        q_s[rows(a, n), c * NC:(c + 1) * NC] = (y * QSCALE).astype(BF16)
                    elif c * NC < 2 * D:
                        k_all[l, pl.ds(pl.multiple_of((ag + 2) * T, T), n * T), c * NC - D:(c + 1) * NC - D] = y.astype(BF16)
                    else:
                        for i in range(n):
                            vt_all[l, ag + 2 + i, c * NC - 2 * D:(c + 1) * NC - 2 * D, :] = y[i * T:(i + 1) * T].T.astype(BF16)
                tasks.append((2 * NC, f))
            return tasks

        def t_out(li, a, n=1):
            tasks = []
            for c in range(D // NC):
                def f(c=c):
                    cs = slice(c * NC, (c + 1) * NC)
                    x_s[rows(a, n), cs] = x_s[rows(a, n), cs] + jnp.dot(o_s[rows(a, n), :], wo_s[li, :, cs], preferred_element_type=F32)
                tasks.append((2 * NC, f))
            return tasks

        def t_attB(r, a):
            tasks = []
            for rg in range(T // RB):
                def f(rg=rg):
                    r0 = a * T + rg * RB
                    qs = [qB[e, r0:r0 + RB, :] for e in range(NG)]
                    Ls = []
                    for w in range(8):
                        R = None
                        for e in range(NG):
                            pr = qs[e] * kB[r, e, pl.ds(r0 + 16 - 2 * w, RB), :]
                            R = pr if R is None else R + pr
                        R = R + pltpu.roll(R, 64, axis=1)
                        R = R + pltpu.roll(R, 32, axis=1)
                        if r0 < 2 * w:
                            pos = lax.broadcasted_iota(jnp.int32, (RB, T), 0) + (t * BM + (r0 - 2 * w))
                            R = jnp.where(pos >= 0, R, NEG)
                        Ls.append(R)
                    m = functools.reduce(jnp.maximum, Ls)
                    ps = [jnp.exp2(L - m) for L in Ls]
                    rl = 1.0 / functools.reduce(jnp.add, ps)
                    ps = [p * rl for p in ps]
                    for e in range(NG):
                        o = None
                        for w in range(8):
                            pr = ps[w] * vB[r, e, pl.ds(r0 + 16 - 2 * w, RB), :]
                            o = pr if o is None else o + pr
                        o_s[r0:r0 + RB, e * T:(e + 1) * T] = o.astype(BF16)
                tasks.append((100, f))
            if a == NSUB - 1:
                def g():
                    for e in range(NG):
                        kB[r, e, 0:16, :] = kB[r, e, BM:BM + 16, :]
                        vB[r, e, 0:16, :] = vB[r, e, BM:BM + 16, :]
                tasks.append((1, g))
            return tasks

        def perm_rows(wt, j):
            for h in range(H):
                tmp[j, pl.ds(h * 33, DH), :] = wt[h * DH:(h + 1) * DH]
            return jnp.concatenate([tmp[j, pl.ds(d, H, stride=33), :] for d in range(DH)], axis=0)

        def permute_qkv(m):
            c0 = m * D
            for i in range(NG):
                wt = wqkv_s[1, i * T:(i + 1) * T, pl.ds(c0, D)].astype(F32).T
                wBT[pl.ds(c0, D), i * T:(i + 1) * T] = perm_rows(wt, i % 4).astype(BF16)

        def permute_o():
            for i in range(NG):
                wo_s[1, :, i * T:(i + 1) * T] = perm_rows(wo_s[1, :, i * T:(i + 1) * T].astype(F32), i % 4).astype(BF16)

        def t_att(r, li, a, parts=False):
            if li == 1:
                return t_attB(r, a)
            isA = li == 0
            l = r
            st_ = {}
            pp_ = {}
            cst = {}

            def s1(g):
                ag = t * NSUB + a
                q4 = pltpu.bitcast(q_s[rows(a), g * T:(g + 1) * T], U32)
                qm = jnp.concatenate([q4 & hmask[h] for h in range(4)], axis=0)
                qm = pltpu.bitcast(qm, BF16)
                if isA:
                    k4 = k_all[l, pl.ds(pl.multiple_of(ag * T, T), 3 * T), g * T:(g + 1) * T]
                else:
                    k4 = k_all[l, pl.ds(pl.multiple_of((ag + 2) * T - 16, 16), T + 16), g * T:(g + 1) * T]
                st_[g] = lax.dot_general(k4, qm, NT, preferred_element_type=F32)

            def s2(g):
                ag = t * NSUB + a
                st = st_.pop(g)
                if isA:
                    bias_far = jnp.where(ag >= 2, 0.0, NEG).astype(F32)
                    bias_mid = jnp.where(ag >= 1, 0.0, NEG).astype(F32)
                    sm = jnp.where(tri4, st[2 * T:], st[:T] + bias_far)
                    smid = st[T:2 * T]
                    m = jnp.maximum(jnp.max(sm, axis=0, keepdims=True), jnp.max(smid, axis=0, keepdims=True) + bias_mid)
                    pm = jnp.exp2(sm - m)
                    pmid = jnp.exp2(smid - (m - bias_mid))
                    lsum = jnp.sum(pm + pmid, axis=0, keepdims=True)
                    pcur = jnp.where(tri4, pm, 0.0)
                    pfar = jnp.where(tri4, 0.0, pm)
                    pp = [jnp.concatenate([pfar[:, h * T:(h + 1) * T], pmid[:, h * T:(h + 1) * T], pcur[:, h * T:(h + 1) * T]], axis=0).astype(BF16) for h in range(4)]
                else:
                    if "b" not in cst:
                        jj = lax.broadcasted_iota(jnp.int32, (T + 16, 4 * T), 0)
                        ii = lax.broadcasted_iota(jnp.int32, (T + 16, 4 * T), 1) & (T - 1)
                        diff = ii - jj + 16
                        validB = (diff >= 0) & (diff <= 14) & ((diff & 1) == 0) & ((jj >= 16) | (ag >= 1))
                        cst["b"] = jnp.where(validB, 0.0, NEG).astype(F32)
                    sm = st + cst["b"]
                    m = jnp.max(sm, axis=0, keepdims=True)
                    pm = jnp.exp2(sm - m)
                    lsum = jnp.sum(pm, axis=0, keepdims=True)
                    pp = [jnp.concatenate([jnp.zeros((T - 16, T), F32), pm[:, h * T:(h + 1) * T]], axis=0).astype(BF16) for h in range(4)]
                pp_[g] = (pp, lsum)

            def s3(g):
                ag = t * NSUB + a
                pp, lsum = pp_.pop(g)
                outs = []
                rl = 1.0 / lsum
                for h in range(4):
                    r0 = g * T + h * DH
                    if isA:
                        vv = jnp.concatenate([vt_all[l, ag + i, r0:r0 + DH, :] for i in range(3)], axis=1)
                    else:
                        vv = jnp.concatenate([vt_all[l, ag + 1 + i, r0:r0 + DH, :] for i in range(2)], axis=1)
                    ot = jnp.dot(vv, pp[h], preferred_element_type=F32)
                    outs.append(ot * rl[:, h * T:(h + 1) * T])
                ot4 = jnp.concatenate(outs, axis=0)
                o_s[rows(a), g * T:(g + 1) * T] = ot4.T.astype(BF16)

            if parts:
                return s1, s2, s3

        def wait(r, i):
            def f():
                @pl.when(jnp.logical_and(t == 0, r == 0))
                def _():
                    for j in {3: (8, 9, 10, 11), 4: (12, 13, 14, 15), 5: (), 6: (6,)}[i]:
                        copy(j).wait()
                    for j in {3: (12, 13, 14, 15), 4: (6, 0, 1, 2, 7), 5: (), 6: ()}[i]:
                        copy(j).start()
            return [(1, f)]

        def prepB(r):
            def f():
                @pl.when(jnp.logical_and(t == 0, r == 0))
                def _():
                    for j in (0, 1, 2, 7):
                        copy(j).wait()
                    for m in range(3):
                        permute_qkv(m)
                    permute_o()
            return [(1, f)]

        def body(r, _):
            seq = []
            npm = D // NC
            for li in range(2):
                pr = [t_proj(r, li, a) for a in range(NSUB)]
                if li == 0:
                    seq += t_ln(0)
                    for m in range(3):
                        seq += wait(r, 3 + m)
                        for a in range(NSUB):
                            seq += pr[a][m * npm:(m + 1) * npm]
                            if m == 0 and a + 1 < NSUB:
                                seq += t_ln(a + 1)
                else:
                    if not PP:
                        seq += prepB(r)
                    for a in range(NSUB):
                        seq += t_ln(a) + pr[a]
                if li == 0 and UNI:
                    fs = [t_att(r, li, a, True) for a in range(NSUB)]
                    n = NSUB * NG
                    for i in range(n + LAG):
                        if i < n:
                            seq.append((1, functools.partial(fs[i // NG][0], i % NG)))
                        if 0 <= i - 1 < n:
                            seq.append((1, functools.partial(fs[(i - 1) // NG][1], (i - 1) % NG)))
                        if 0 <= i - LAG < n:
                            seq.append((1, functools.partial(fs[(i - LAG) // NG][2], (i - LAG) % NG)))
                        if PP and i == PP:
                            seq += prepB(r)
                else:
                    for a in range(NSUB):
                        seq += t_att(r, li, a)
                if li == 0:
                    seq += wait(r, 6)
                for a in range(NSUB):
                    seq += t_out(li, a)
            for _, f in seq:
                f()
            return 0
        lax.fori_loop(0, 2, body, 0)
        out_ref[...] = x_s[...].astype(out_ref.dtype)

    def run(A_x, A_wqkv, A_wo, B_x, B_wqkv, B_wo):
        x = A_x.reshape(S, D)
        anyspec = pl.BlockSpec(memory_space=pl.ANY)
        kw = {}
        if FLAGS:
            kw["flags"] = FLAGS
        out = pl.pallas_call(
            kernel,
            grid=(NS,),
            in_specs=[pl.BlockSpec((BM, D), lambda i: (i, 0)), anyspec, anyspec, anyspec, anyspec],
            out_specs=pl.BlockSpec((BM, D), lambda i: (i, 0)),
            out_shape=jax.ShapeDtypeStruct((S, D), A_x.dtype),
            scratch_shapes=[
                pltpu.VMEM((2, D, 3 * D), BF16), pltpu.VMEM((2, D, D), BF16),
                pltpu.VMEM((BM, D), F32), pltpu.VMEM((BM, D), BF16), pltpu.VMEM((BM, D), BF16), pltpu.VMEM((BM, D), BF16),
                pltpu.VMEM((2, (NB + 2) * T, D), BF16), pltpu.VMEM((2, NB + 2, D, T), BF16),
                pltpu.VMEM((NG, BM, T), F32), pltpu.VMEM((2, NG, BM + 16, T), F32), pltpu.VMEM((2, NG, BM + 16, T), F32),
                pltpu.VMEM((4, 33 * H, T), F32), pltpu.VMEM((3 * D, D), BF16),
                pltpu.SemaphoreType.DMA((16,))],
            compiler_params=pltpu.CompilerParams(
                dimension_semantics=("arbitrary",), vmem_limit_bytes=110 * 1024 * 1024, **kw),
        )(x, A_wqkv, A_wo, B_wqkv, B_wo)
        return out.reshape(1, S, D)
    return run


@jax.jit
def pallas_interleave_layers__sliding_block__sliding_local_dilated__prompt_kernel(
    A_x, A_wqkv, A_wo, B_x, B_wqkv, B_wo):
    return _make()(A_x, A_wqkv, A_wo, B_x, B_wqkv, B_wo)
```
